```python
import os as _os
_os.environ.setdefault("JAX_PLATFORMS", "cpu")
import jax
import jax.numpy as jnp

def _softmax(x, axis=-1):
    return jax.nn.softmax(x, axis=axis)
def _gelu(x):
    return jax.nn.gelu(x, approximate=True)
def _silu(x):
    return jax.nn.silu(x)
def _sigmoid(x):
    return jax.nn.sigmoid(x)
def _layernorm(x, axis=-1, eps=1e-5):
    m = jnp.mean(x, axis=axis, keepdims=True)
    v = jnp.var(x, axis=axis, keepdims=True)
    return (x - m) / jnp.sqrt(v + eps)
def _scatter_add(tgt, idx, src, axis=0):
    return tgt.at[idx].add(src)
def _segment_sum(src, seg, n):
    return jax.ops.segment_sum(src, seg, n)
class _Rng:
    def __init__(self, key):
        self._k = key
    def _next(self):
        self._k, sub = jax.random.split(self._k)
        return sub
    def normal(self, shape):
        return jax.random.normal(self._next(), shape, dtype=jnp.bfloat16)
    def randint(self, lo, hi, shape):
        return jax.random.randint(self._next(), shape, lo, hi, dtype=jnp.int32)
    def uniform(self, shape, lo=0.0, hi=1.0):
        return jax.random.uniform(self._next(), shape, jnp.bfloat16, lo, hi)
    def permutation(self, n):
        return jax.random.permutation(self._next(), n)


kernel_name = 'concat_heads__sliding_local_dilated__sliding_block__prompt'

def setup_inputs():
    _rng = _Rng(jax.random.key(int.from_bytes(__import__("os").urandom(4), "little")))
    _w = (lambda a: (lambda t: t.astype(jnp.bfloat16) if jnp.issubdtype(t.dtype, jnp.floating) else t)(jnp.asarray(a)))
    def _A_setup():
        B, S, D = 1, 2048, 1024
        return {
            "x": _w((lambda *s: _rng.normal(s) * 0.2)(B, S, D)),
            "wqkv": _w((lambda *s: _rng.normal(s) * 0.2)(D, 3 * D)),
            "wo": _w((lambda *s: _rng.normal(s) * 0.05)(D, D)),
        }
    _A_in = _A_setup()

    def _B_setup():
        B, S, D = 1, 2048, 1024
        return {
            "x": _w((lambda *s: _rng.normal(s) * 0.2)(B, S, D)),
            "wqkv": _w((lambda *s: _rng.normal(s) * 0.2)(D, 3 * D)),
            "wo": _w((lambda *s: _rng.normal(s) * 0.05)(D, D)),
        }
    _B_in = _B_setup()

    return {
        "A_x": _A_in["x"],
        "A_wqkv": _A_in["wqkv"],
        "A_wo": _A_in["wo"],
        "B_x": _B_in["x"],
        "B_wqkv": _B_in["wqkv"],
        "B_wo": _B_in["wo"],
    }

def reference(A_x, A_wqkv, A_wo, B_x, B_wqkv, B_wo):
    def _A_ref(x, wqkv, wo):
        B, S, D = x.shape
        H = 32; Dh = D // H
        W, dil = 8, 2
        qkv = (lambda x, *d: x.transpose(*d))((x @ wqkv).reshape(B, S, 3, H, Dh), 2, 0, 3, 1, 4)
        q, k, v = qkv[0], qkv[1], qkv[2]
        scale = Dh ** -0.5
        pos = jnp.arange(S)
        off = jnp.arange(W) * dil
        idx = pos[:, None] - off[None, :]
        mask = idx >= 0
        idx_c = jnp.where(mask, idx, 0).reshape(-1)
        kg = k[:, :, idx_c, :].reshape(B, H, S, W, Dh)
        vg = v[:, :, idx_c, :].reshape(B, H, S, W, Dh)
        logits = jnp.einsum("bhsd,bhswd->bhsw", q, kg) * scale
        logits = jnp.where(mask[None, None, :, :], logits, -1e9)
        attn = _softmax(logits, axis=-1)
        o = jnp.einsum("bhsw,bhswd->bhsd", attn, vg)
        return (lambda x, *d: x.transpose(*d))(o, 0, 2, 1, 3).reshape(B, S, D) @ wo

    def _B_ref(x, wqkv, wo):
        B, S, D = x.shape
        H = 32; Dh = D // H; W = 256
        qkv = (lambda x, *d: x.transpose(*d))((x @ wqkv).reshape(B, S, 3, H, Dh), 2, 0, 3, 1, 4)
        q, k, v = qkv[0], qkv[1], qkv[2]
        scores = jnp.einsum("bhqd,bhkd->bhqk", q, k) * (Dh ** -0.5)
        idx = jnp.arange(S)
        mask = (idx[:, None] - idx[None, :] >= 0) & (idx[:, None] - idx[None, :] < W)
        scores = jnp.where(mask[None, None], scores, -1e9)
        p = _softmax(scores, axis=-1)
        o = jnp.einsum("bhqk,bhkd->bhqd", p, v)
        return (lambda x, *d: x.transpose(*d))(o, 0, 2, 1, 3).reshape(B, S, D) @ wo

    a = _A_ref(A_x, A_wqkv, A_wo)
    b = _B_ref(B_x, B_wqkv, B_wo)
    return jnp.concatenate([a, b], axis=-1)
```

```python
import functools
import jax
import jax.numpy as jnp
from jax import lax
import jax.experimental.pallas as pl
import jax.experimental.pallas.tpu as pltpu

S, D, H, DH = 2048, 1024, 32, 32
TQ = 256
QB = 128
NG = D // 128
WB = 256
HALO_A = 128
NT = (((1,), (1,)), ((), ()))
NEG = -1e9


def _attn_group(q4, kw, vw, mask):
    lane = lax.broadcasted_iota(jnp.int32, (QB, 128), 1) // DH
    zero = jnp.zeros_like(q4)
    qs = jnp.concatenate([jnp.where(lane == h, q4, zero) for h in range(4)], axis=0)
    s = lax.dot_general(qs, kw, NT, preferred_element_type=jnp.float32)
    s = jnp.where(mask, s, NEG)
    m = jnp.max(s, axis=-1, keepdims=True)
    p = jnp.exp(s - m)
    l = jnp.sum(p, axis=-1, keepdims=True)
    o = jnp.dot(p.astype(jnp.bfloat16), vw, preferred_element_type=jnp.float32)
    o = o / l
    out = o[0:QB]
    for h in range(1, 4):
        out = jnp.where(lane == h, o[h * QB:(h + 1) * QB], out)
    return out


def _kernel(ax_ref, awqkv_ref, awo_ref, bx_ref, bwqkv_ref, bwo_ref, out_ref,
            q_scr, ka_scr, va_scr, kb_scr, vb_scr, o_scr):
    i = pl.program_id(0)
    scale = DH ** -0.5

    @pl.when(i == 0)
    def _():
        ka_scr[0:HALO_A, :] = jnp.zeros((HALO_A, D), jnp.bfloat16)
        va_scr[0:HALO_A, :] = jnp.zeros((HALO_A, D), jnp.bfloat16)
        kb_scr[0:WB, :] = jnp.zeros((WB, D), jnp.bfloat16)
        vb_scr[0:WB, :] = jnp.zeros((WB, D), jnp.bfloat16)

    def branch(x_ref, wqkv_ref, wo_ref, k_scr, v_scr, halo, tk, maskfn, col0):
        x = x_ref[...]
        q = jnp.dot(x, wqkv_ref[:, 0:D], preferred_element_type=jnp.float32)
        q_scr[...] = (q * scale).astype(jnp.bfloat16)
        r0 = pl.multiple_of(i * TQ + halo, 128)
        k_scr[pl.ds(r0, TQ), :] = jnp.dot(x, wqkv_ref[:, D:2 * D], preferred_element_type=jnp.float32).astype(jnp.bfloat16)
        v_scr[pl.ds(r0, TQ), :] = jnp.dot(x, wqkv_ref[:, 2 * D:3 * D], preferred_element_type=jnp.float32).astype(jnp.bfloat16)
        for qb in range(TQ // QB):
            q0 = i * TQ + qb * QB
            row = lax.broadcasted_iota(jnp.int32, (4 * QB, tk), 0) % QB
            col = lax.broadcasted_iota(jnp.int32, (4 * QB, tk), 1)
            d = row - col + halo
            mask = maskfn(d) & (col + (q0 - halo) >= 0)
            w0 = pl.multiple_of(q0, 128)

            def body(g, carry):
                c0 = pl.multiple_of(g * 128, 128)
                q4 = q_scr[qb * QB:(qb + 1) * QB, pl.ds(c0, 128)]
                kw = k_scr[pl.ds(w0, tk), pl.ds(c0, 128)]
                vw = v_scr[pl.ds(w0, tk), pl.ds(c0, 128)]
                o_scr[qb * QB:(qb + 1) * QB, pl.ds(c0, 128)] = _attn_group(q4, kw, vw, mask).astype(jnp.bfloat16)
                return carry
            lax.fori_loop(0, NG, body, 0)
        out_ref[:, col0:col0 + D] = jnp.dot(o_scr[...], wo_ref[...], preferred_element_type=jnp.float32).astype(out_ref.dtype)

    branch(ax_ref, awqkv_ref, awo_ref, ka_scr, va_scr, HALO_A, HALO_A + QB,
           lambda d: (d >= 0) & (d <= 14) & (d % 2 == 0), 0)
    branch(bx_ref, bwqkv_ref, bwo_ref, kb_scr, vb_scr, WB, WB + QB,
           lambda d: (d >= 0) & (d < WB), D)


@jax.jit
def pallas_concat_heads__sliding_local_dilated__sliding_block__prompt_kernel(
    A_x, A_wqkv, A_wo, B_x, B_wqkv, B_wo):
    ax = A_x.reshape(S, D)
    bx = B_x.reshape(S, D)
    xspec = pl.BlockSpec((TQ, D), lambda i: (i, 0))
    w1 = pl.BlockSpec((D, 3 * D), lambda i: (0, 0), pipeline_mode=pl.Buffered(1))
    w2 = pl.BlockSpec((D, D), lambda i: (0, 0), pipeline_mode=pl.Buffered(1))
    out = pl.pallas_call(
        _kernel,
        grid=(S // TQ,),
        in_specs=[xspec, w1, w2, xspec, w1, w2],
        out_specs=pl.BlockSpec((TQ, 2 * D), lambda i: (i, 0)),
        out_shape=jax.ShapeDtypeStruct((S, 2 * D), jnp.bfloat16),
        scratch_shapes=[
            pltpu.VMEM((TQ, D), jnp.bfloat16),
            pltpu.VMEM((S + HALO_A, D), jnp.bfloat16),
            pltpu.VMEM((S + HALO_A, D), jnp.bfloat16),
            pltpu.VMEM((S + WB, D), jnp.bfloat16),
            pltpu.VMEM((S + WB, D), jnp.bfloat16),
            pltpu.VMEM((TQ, D), jnp.bfloat16),
        ],
        compiler_params=pltpu.CompilerParams(
            dimension_semantics=("arbitrary",),
            vmem_limit_bytes=100 * 1024 * 1024),
    )(ax, A_wqkv, A_wo, bx, B_wqkv, B_wo)
    return out.reshape(1, S, 2 * D)
```

```python
import functools
import math
import jax
import jax.numpy as jnp
from jax import lax
import jax.experimental.pallas as pl
import jax.experimental.pallas.tpu as pltpu

S, D, H, DH = 2048, 1024, 32, 32
TQ = 256
NG = D // 128
WB = 256
HALO_A = 32
NT = (((1,), (1,)), ((), ()))
NEG = -1e9
QSCALE = DH ** -0.5 * math.log2(math.e)
NSLAB = TQ // 32
NC = NSLAB + WB // 32


def _stack4(blk, hmasks):
    w = pltpu.bitcast(blk, jnp.uint32)
    return pltpu.bitcast(jnp.concatenate([w & hm for hm in hmasks], axis=0), jnp.bfloat16)


def _segmax(mm, lane_h):
    mseg = mm
    for h in range(4):
        mh = jnp.max(jnp.where(lane_h == h, mm, -jnp.inf), axis=1, keepdims=True)
        mseg = jnp.where(lane_h == h, mh, mseg)
    return mseg


def _segsum(mm, lane_h):
    out = mm
    for h in range(4):
        mh = jnp.sum(jnp.where(lane_h == h, mm, 0.0), axis=1, keepdims=True)
        out = jnp.where(lane_h == h, mh, out)
    return out


def _phase1(q, k_scr, c0, chunks, slab, nslab, hmasks):
    m = [None] * nslab
    svals = []
    for (kr, t_lo, t_hi, add, masks) in chunks:
        ks = _stack4(k_scr[pl.ds(kr, 32), c0:c0 + 128], hmasks)
        s = lax.dot_general(q[slab * t_lo:slab * (t_hi + 1)], ks, NT, preferred_element_type=jnp.float32)
        if add is not None:
            s = s + add
        slabs = []
        for t in range(t_lo, t_hi + 1):
            sl = s[slab * (t - t_lo):slab * (t - t_lo + 1)]
            if t in masks:
                sl = jnp.where(masks[t], sl, NEG)
            m[t] = sl if m[t] is None else jnp.maximum(m[t], sl)
            slabs.append(sl)
        svals.append(slabs)
    return svals, m


def _phase2(state, v_scr, c0, chunks, slab, nslab, hmasks, lane_hT, bd_ones):
    svals, m = state
    mseg = _segmax(jnp.concatenate(m, axis=0), lane_hT)
    psum = [None] * nslab
    oacc = [None] * nslab
    for ci, (kr, t_lo, t_hi, add, masks) in enumerate(chunks):
        vs = _stack4(v_scr[pl.ds(kr, 32), c0:c0 + 128], hmasks)
        ps = []
        for t in range(t_lo, t_hi + 1):
            p = jnp.exp2(svals[ci][t - t_lo] - mseg[slab * t:slab * (t + 1)])
            psum[t] = p if psum[t] is None else psum[t] + p
            ps.append(p.astype(jnp.bfloat16))
        pb = jnp.concatenate(ps, axis=0)
        o = jnp.dot(pb, vs, preferred_element_type=jnp.float32)
        for t in range(t_lo, t_hi + 1):
            ot = o[slab * (t - t_lo):slab * (t - t_lo + 1)]
            oacc[t] = ot if oacc[t] is None else oacc[t] + ot
    l = _segsum(jnp.concatenate(psum, axis=0), lane_hT)
    return (jnp.concatenate(oacc, axis=0) * pl.reciprocal(l, approx=True)).astype(jnp.bfloat16)


def _kernel(ax_ref, awqkv_hbm, awo_hbm, bx_ref, bwqkv_hbm, bwo_hbm, out_ref,
            awqkv_ref, awo_ref, bwqkv_ref, bwo_ref, sems,
            qa_scr, ka_scr, va_scr, kb_scr, vb_scr, oa_scr, qb_scr, ob_scr):
    i = pl.program_id(0)

    def wcopy(n):
        if n < 3:
            return pltpu.make_async_copy(awqkv_hbm.at[:, n * D:(n + 1) * D], awqkv_ref.at[:, n * D:(n + 1) * D], sems.at[n])
        if n == 3:
            return pltpu.make_async_copy(awo_hbm, awo_ref, sems.at[n])
        if n < 7:
            return pltpu.make_async_copy(bwqkv_hbm.at[:, (n - 4) * D:(n - 3) * D], bwqkv_ref.at[:, (n - 4) * D:(n - 3) * D], sems.at[n])
        return pltpu.make_async_copy(bwo_hbm, bwo_ref, sems.at[n])

    @pl.when(i == 0)
    def _():
        for n in (0, 1, 2):
            wcopy(n).start()
        ka_scr[0:HALO_A, :] = jnp.zeros((HALO_A, D), jnp.bfloat16)
        va_scr[0:HALO_A, :] = jnp.zeros((HALO_A, D), jnp.bfloat16)
        kb_scr[0:WB, :] = jnp.zeros((WB, D), jnp.bfloat16)
        vb_scr[0:WB, :] = jnp.zeros((WB, D), jnp.bfloat16)
        for n in (0, 1, 2):
            wcopy(n).wait()
        for n in (4, 5, 6, 3, 7):
            wcopy(n).start()

    def wait(ns):
        @pl.when(i == 0)
        def _():
            for n in ns:
                wcopy(n).wait()

    lane16 = lax.broadcasted_iota(jnp.int32, (16, 128), 1)
    hmasks = [jnp.where(lane16 // DH == h, jnp.uint32(0xFFFFFFFF), jnp.uint32(0)) for h in range(4)]
    pen = jnp.where(i == 0, NEG, 0.0).astype(jnp.float32)
    rr = lax.broadcasted_iota(jnp.int32, (128, 128), 0) // DH
    cc = lax.broadcasted_iota(jnp.int32, (128, 128), 1) // DH
    bd_ones = jnp.where(rr == cc, 1.0, 0.0).astype(jnp.bfloat16)
    lane_hT = lax.broadcasted_iota(jnp.int32, (TQ, 128), 1) // DH

    xa = ax_ref[...]
    ra = pl.multiple_of(i * TQ + HALO_A, 32)
    qa_scr[...] = (jnp.dot(xa, awqkv_ref[:, 0:D], preferred_element_type=jnp.float32) * QSCALE).astype(jnp.bfloat16)
    ka_scr[pl.ds(ra, TQ), :] = jnp.dot(xa, awqkv_ref[:, D:2 * D], preferred_element_type=jnp.float32).astype(jnp.bfloat16)
    va_scr[pl.ds(ra, TQ), :] = jnp.dot(xa, awqkv_ref[:, 2 * D:3 * D], preferred_element_type=jnp.float32).astype(jnp.bfloat16)

    j16 = lane16 % DH
    r16 = lax.broadcasted_iota(jnp.int32, (16, 128), 0)
    amask = []
    for u in range(3):
        d = r16 + 16 * u - j16
        amask.append((d >= 0) & (d <= 14) & ((d & 1) == 0))
    nsA = TQ // 16
    chunksA = []
    for c in range(TQ // 32 + 1):
        kr = pl.multiple_of(i * TQ + 32 * c, 32)
        t_lo = max(0, 2 * (c - 1))
        t_hi = min(nsA - 1, 2 * c)
        masks = {t: amask[t - 2 * (c - 1)] for t in range(t_lo, t_hi + 1)}
        chunksA.append((kr, t_lo, t_hi, pen if c == 0 else None, masks))

    j32 = lax.broadcasted_iota(jnp.int32, (32, 128), 1) % DH
    r32 = lax.broadcasted_iota(jnp.int32, (32, 128), 0)
    tril = r32 >= j32
    triu = r32 < j32
    chunksB = []
    for c in range(NC):
        kr = pl.multiple_of(i * TQ + 32 * c, 32)
        t_lo = max(0, c - 8)
        t_hi = min(NSLAB - 1, c)
        masks = {}
        if c - 8 >= 0:
            masks[c - 8] = tril
        if c <= NSLAB - 1:
            masks[c] = triu
        chunksB.append((kr, t_lo, t_hi, pen if c < 8 else None, masks))

    wait([4, 5, 6])
    xb = bx_ref[...]
    rb = pl.multiple_of(i * TQ + WB, 32)
    for g in range(NG):
        c0 = g * 128
        st = _phase1(qa_scr[:, c0:c0 + 128], ka_scr, c0, chunksA, 16, nsA, hmasks)
        for cb in range(3 * g, 3 * g + 3):
            y = jnp.dot(xb, bwqkv_ref[:, cb * 128:(cb + 1) * 128], preferred_element_type=jnp.float32)
            which, col = cb // NG, (cb % NG) * 128
            if which == 0:
                qb_scr[:, col:col + 128] = (y * QSCALE).astype(jnp.bfloat16)
            elif which == 1:
                kb_scr[pl.ds(rb, TQ), col:col + 128] = y.astype(jnp.bfloat16)
            else:
                vb_scr[pl.ds(rb, TQ), col:col + 128] = y.astype(jnp.bfloat16)
        oa_scr[:, c0:c0 + 128] = _phase2(st, va_scr, c0, chunksA, 16, nsA, hmasks, lane_hT, bd_ones)
    wait([3, 7])

    oa = oa_scr[...]
    st = _phase1(qb_scr[:, 0:128], kb_scr, 0, chunksB, 32, NSLAB, hmasks)
    for g in range(NG):
        c0 = g * 128
        out_ref[:, c0:c0 + 128] = jnp.dot(oa, awo_ref[:, c0:c0 + 128], preferred_element_type=jnp.float32).astype(out_ref.dtype)
        if g + 1 < NG:
            st_next = _phase1(qb_scr[:, c0 + 128:c0 + 256], kb_scr, c0 + 128, chunksB, 32, NSLAB, hmasks)
        ob_scr[:, c0:c0 + 128] = _phase2(st, vb_scr, c0, chunksB, 32, NSLAB, hmasks, lane_hT, bd_ones)
        st = st_next
    out_ref[:, D:2 * D] = jnp.dot(ob_scr[...], bwo_ref[...], preferred_element_type=jnp.float32).astype(out_ref.dtype)


@jax.jit
def pallas_concat_heads__sliding_local_dilated__sliding_block__prompt_kernel(
    A_x, A_wqkv, A_wo, B_x, B_wqkv, B_wo):
    ax = A_x.reshape(S, D)
    bx = B_x.reshape(S, D)
    xspec = pl.BlockSpec((TQ, D), lambda i: (i, 0))
    anyspec = pl.BlockSpec(memory_space=pl.ANY)
    out = pl.pallas_call(
        _kernel,
        grid=(S // TQ,),
        in_specs=[xspec, anyspec, anyspec, xspec, anyspec, anyspec],
        out_specs=pl.BlockSpec((TQ, 2 * D), lambda i: (i, 0)),
        out_shape=jax.ShapeDtypeStruct((S, 2 * D), jnp.bfloat16),
        scratch_shapes=[
            pltpu.VMEM((D, 3 * D), jnp.bfloat16),
            pltpu.VMEM((D, D), jnp.bfloat16),
            pltpu.VMEM((D, 3 * D), jnp.bfloat16),
            pltpu.VMEM((D, D), jnp.bfloat16),
            pltpu.SemaphoreType.DMA((8,)),
            pltpu.VMEM((TQ, D), jnp.bfloat16),
            pltpu.VMEM((S + HALO_A, D), jnp.bfloat16),
            pltpu.VMEM((S + HALO_A, D), jnp.bfloat16),
            pltpu.VMEM((S + WB, D), jnp.bfloat16),
            pltpu.VMEM((S + WB, D), jnp.bfloat16),
            pltpu.VMEM((TQ, D), jnp.bfloat16),
            pltpu.VMEM((TQ, D), jnp.bfloat16),
            pltpu.VMEM((TQ, D), jnp.bfloat16),
        ],
        compiler_params=pltpu.CompilerParams(
            dimension_semantics=("arbitrary",),
            vmem_limit_bytes=100 * 1024 * 1024),
    )(ax, A_wqkv, A_wo, bx, B_wqkv, B_wo)
    return out.reshape(1, S, 2 * D)
```

```python
import math
import jax
import jax.numpy as jnp
from jax import lax
import jax.experimental.pallas as pl
import jax.experimental.pallas.tpu as pltpu

S, D, DH = 2048, 1024, 32
TQ = 256
NG = D // 128
WB = 256
HALO_A = 32
NT = (((1,), (1,)), ((), ()))
NEG = -1e9
QSCALE = DH ** -0.5 * math.log2(math.e)
NSLAB = TQ // 32
NC = NSLAB + WB // 32


def _stack4(blk, hmasks):
    w = pltpu.bitcast(blk, jnp.uint32)
    return pltpu.bitcast(jnp.concatenate([w & hm for hm in hmasks], axis=0), jnp.bfloat16)


def _segmax(x, lane_h):
    out = x
    for h in range(4):
        mh = jnp.max(jnp.where(lane_h == h, x, -jnp.inf), axis=1, keepdims=True)
        out = jnp.where(lane_h == h, mh, out)
    return out


def _segsum(x, lane_h):
    out = x
    for h in range(4):
        sh = jnp.sum(jnp.where(lane_h == h, x, 0.0), axis=1, keepdims=True)
        out = jnp.where(lane_h == h, sh, out)
    return out


def _phase1(q, k_scr, c0, chunks, slab, nslab, hmasks):
    m = [None] * nslab
    svals = []
    for (kr, t_lo, t_hi, add, masks) in chunks:
        ks = _stack4(k_scr[pl.ds(kr, 32), c0:c0 + 128], hmasks)
        s = lax.dot_general(q[slab * t_lo:slab * (t_hi + 1)], ks, NT, preferred_element_type=jnp.float32)
        if add is not None:
            s = s + add
        slabs = []
        for t in range(t_lo, t_hi + 1):
            sl = s[slab * (t - t_lo):slab * (t - t_lo + 1)]
            if t in masks:
                sl = jnp.where(masks[t], sl, NEG)
            m[t] = sl if m[t] is None else jnp.maximum(m[t], sl)
            slabs.append(sl)
        svals.append(slabs)
    return svals, m


def _phase2(state, v_scr, c0, chunks, slab, nslab, hmasks, lane_hT):
    svals, m = state
    mseg = _segmax(jnp.concatenate(m, axis=0), lane_hT)
    psum = [None] * nslab
    oacc = [None] * nslab
    for ci, (kr, t_lo, t_hi, add, masks) in enumerate(chunks):
        vs = _stack4(v_scr[pl.ds(kr, 32), c0:c0 + 128], hmasks)
        ps = []
        for t in range(t_lo, t_hi + 1):
            p = jnp.exp2(svals[ci][t - t_lo] - mseg[slab * t:slab * (t + 1)])
            psum[t] = p if psum[t] is None else psum[t] + p
            ps.append(p.astype(jnp.bfloat16))
        pb = jnp.concatenate(ps, axis=0)
        o = jnp.dot(pb, vs, preferred_element_type=jnp.float32)
        for t in range(t_lo, t_hi + 1):
            ot = o[slab * (t - t_lo):slab * (t - t_lo + 1)]
            oacc[t] = ot if oacc[t] is None else oacc[t] + ot
    l = _segsum(jnp.concatenate(psum, axis=0), lane_hT)
    return (jnp.concatenate(oacc, axis=0) * pl.reciprocal(l, approx=True)).astype(jnp.bfloat16)


def _kernel(ax_ref, awqkv_hbm, awo_hbm, bx_ref, bwqkv_hbm, bwo_hbm, out_ref,
            awqkv_ref, awo_ref, bwqkv_ref, bwo_ref, sems,
            qa_scr, ka_scr, va_scr, kb_scr, vb_scr, oa_scr, qb_scr, ob_scr):
    i = pl.program_id(0)

    def wcopy(n):
        if n < 3:
            return pltpu.make_async_copy(awqkv_hbm.at[:, n * D:(n + 1) * D],
                                         awqkv_ref.at[:, n * D:(n + 1) * D], sems.at[n])
        if n == 3:
            return pltpu.make_async_copy(awo_hbm, awo_ref, sems.at[n])
        if n < 7:
            return pltpu.make_async_copy(bwqkv_hbm.at[:, (n - 4) * D:(n - 3) * D],
                                         bwqkv_ref.at[:, (n - 4) * D:(n - 3) * D], sems.at[n])
        return pltpu.make_async_copy(bwo_hbm, bwo_ref, sems.at[n])

    @pl.when(i == 0)
    def _():
        for n in (0, 1, 2):
            wcopy(n).start()
        ka_scr[0:HALO_A, :] = jnp.zeros((HALO_A, D), jnp.bfloat16)
        va_scr[0:HALO_A, :] = jnp.zeros((HALO_A, D), jnp.bfloat16)
        kb_scr[0:WB, :] = jnp.zeros((WB, D), jnp.bfloat16)
        vb_scr[0:WB, :] = jnp.zeros((WB, D), jnp.bfloat16)
        for n in (0, 1, 2):
            wcopy(n).wait()
        for n in (4, 5, 6, 3, 7):
            wcopy(n).start()

    def wait(ns):
        @pl.when(i == 0)
        def _():
            for n in ns:
                wcopy(n).wait()

    lane16 = lax.broadcasted_iota(jnp.int32, (16, 128), 1)
    hmasks = [jnp.where(lane16 // DH == h, jnp.uint32(0xFFFFFFFF), jnp.uint32(0)) for h in range(4)]
    pen = jnp.where(i == 0, NEG, 0.0).astype(jnp.float32)
    lane_hT = lax.broadcasted_iota(jnp.int32, (TQ, 128), 1) // DH

    xa = ax_ref[...]
    ra = pl.multiple_of(i * TQ + HALO_A, 32)
    qa_scr[...] = (jnp.dot(xa, awqkv_ref[:, 0:D], preferred_element_type=jnp.float32) * QSCALE).astype(jnp.bfloat16)
    ka_scr[pl.ds(ra, TQ), :] = jnp.dot(xa, awqkv_ref[:, D:2 * D], preferred_element_type=jnp.float32).astype(jnp.bfloat16)
    va_scr[pl.ds(ra, TQ), :] = jnp.dot(xa, awqkv_ref[:, 2 * D:3 * D], preferred_element_type=jnp.float32).astype(jnp.bfloat16)

    j16 = lane16 % DH
    r16 = lax.broadcasted_iota(jnp.int32, (16, 128), 0)
    amask = []
    for u in range(3):
        d = r16 + 16 * u - j16
        amask.append((d >= 0) & (d <= 14) & ((d & 1) == 0))
    nsA = TQ // 16
    chunksA = []
    for c in range(TQ // 32 + 1):
        kr = pl.multiple_of(i * TQ + 32 * c, 32)
        t_lo = max(0, 2 * (c - 1))
        t_hi = min(nsA - 1, 2 * c)
        masks = {t: amask[t - 2 * (c - 1)] for t in range(t_lo, t_hi + 1)}
        chunksA.append((kr, t_lo, t_hi, pen if c == 0 else None, masks))

    j32 = lax.broadcasted_iota(jnp.int32, (32, 128), 1) % DH
    r32 = lax.broadcasted_iota(jnp.int32, (32, 128), 0)
    tril = r32 >= j32
    triu = r32 < j32
    chunksB = []
    for c in range(NC):
        kr = pl.multiple_of(i * TQ + 32 * c, 32)
        t_lo = max(0, c - 8)
        t_hi = min(NSLAB - 1, c)
        masks = {}
        if c - 8 >= 0:
            masks[c - 8] = tril
        if c <= NSLAB - 1:
            masks[c] = triu
        chunksB.append((kr, t_lo, t_hi, pen if c < 8 else None, masks))

    wait([4, 5, 6])
    xb = bx_ref[...]
    rb = pl.multiple_of(i * TQ + WB, 32)
    for g in range(NG):
        c0 = g * 128
        st = _phase1(qa_scr[:, c0:c0 + 128], ka_scr, c0, chunksA, 16, nsA, hmasks)
        for cb in range(3 * g, 3 * g + 3):
            y = jnp.dot(xb, bwqkv_ref[:, cb * 128:(cb + 1) * 128], preferred_element_type=jnp.float32)
            which, col = cb // NG, (cb % NG) * 128
            if which == 0:
                qb_scr[:, col:col + 128] = (y * QSCALE).astype(jnp.bfloat16)
            elif which == 1:
                kb_scr[pl.ds(rb, TQ), col:col + 128] = y.astype(jnp.bfloat16)
            else:
                vb_scr[pl.ds(rb, TQ), col:col + 128] = y.astype(jnp.bfloat16)
        oa_scr[:, c0:c0 + 128] = _phase2(st, va_scr, c0, chunksA, 16, nsA, hmasks, lane_hT)
    wait([3, 7])

    oa = oa_scr[...]
    for g in range(NG):
        c0 = g * 128
        st = _phase1(qb_scr[:, c0:c0 + 128], kb_scr, c0, chunksB, 32, NSLAB, hmasks)
        out_ref[:, c0:c0 + 128] = jnp.dot(oa, awo_ref[:, c0:c0 + 128],
                                          preferred_element_type=jnp.float32).astype(out_ref.dtype)
        ob_scr[:, c0:c0 + 128] = _phase2(st, vb_scr, c0, chunksB, 32, NSLAB, hmasks, lane_hT)
    out_ref[:, D:2 * D] = jnp.dot(ob_scr[...], bwo_ref[...],
                                  preferred_element_type=jnp.float32).astype(out_ref.dtype)


@jax.jit
def pallas_concat_heads__sliding_local_dilated__sliding_block__prompt_kernel(
    A_x: jax.Array,
    A_wqkv: jax.Array,
    A_wo: jax.Array,
    B_x: jax.Array,
    B_wqkv: jax.Array,
    B_wo: jax.Array,
):
    ax = A_x.reshape(S, D)
    bx = B_x.reshape(S, D)
    xspec = pl.BlockSpec((TQ, D), lambda i: (i, 0))
    anyspec = pl.BlockSpec(memory_space=pl.ANY)
    out = pl.pallas_call(
        _kernel,
        grid=(S // TQ,),
        in_specs=[xspec, anyspec, anyspec, xspec, anyspec, anyspec],
        out_specs=pl.BlockSpec((TQ, 2 * D), lambda i: (i, 0)),
        out_shape=jax.ShapeDtypeStruct((S, 2 * D), jnp.bfloat16),
        scratch_shapes=[
            pltpu.VMEM((D, 3 * D), jnp.bfloat16),
            pltpu.VMEM((D, D), jnp.bfloat16),
            pltpu.VMEM((D, 3 * D), jnp.bfloat16),
            pltpu.VMEM((D, D), jnp.bfloat16),
            pltpu.SemaphoreType.DMA((8,)),
            pltpu.VMEM((TQ, D), jnp.bfloat16),
            pltpu.VMEM((S + HALO_A, D), jnp.bfloat16),
            pltpu.VMEM((S + HALO_A, D), jnp.bfloat16),
            pltpu.VMEM((S + WB, D), jnp.bfloat16),
            pltpu.VMEM((S + WB, D), jnp.bfloat16),
            pltpu.VMEM((TQ, D), jnp.bfloat16),
            pltpu.VMEM((TQ, D), jnp.bfloat16),
            pltpu.VMEM((TQ, D), jnp.bfloat16),
        ],
        compiler_params=pltpu.CompilerParams(
            dimension_semantics=("arbitrary",),
            vmem_limit_bytes=100 * 1024 * 1024),
    )(ax, A_wqkv, A_wo, bx, B_wqkv, B_wo)
    return out.reshape(1, S, 2 * D)
```
